```python
import os as _os
_os.environ.setdefault("JAX_PLATFORMS", "cpu")
import jax
import jax.numpy as jnp

def _softmax(x, axis=-1):
    return jax.nn.softmax(x, axis=axis)
def _gelu(x):
    return jax.nn.gelu(x, approximate=True)
def _silu(x):
    return jax.nn.silu(x)
def _sigmoid(x):
    return jax.nn.sigmoid(x)
def _layernorm(x, axis=-1, eps=1e-5):
    m = jnp.mean(x, axis=axis, keepdims=True)
    v = jnp.var(x, axis=axis, keepdims=True)
    return (x - m) / jnp.sqrt(v + eps)
def _scatter_add(tgt, idx, src, axis=0):
    return tgt.at[idx].add(src)
def _segment_sum(src, seg, n):
    return jax.ops.segment_sum(src, seg, n)
class _Rng:
    def __init__(self, key):
        self._k = key
    def _next(self):
        self._k, sub = jax.random.split(self._k)
        return sub
    def normal(self, shape):
        return jax.random.normal(self._next(), shape, dtype=jnp.bfloat16)
    def randint(self, lo, hi, shape):
        return jax.random.randint(self._next(), shape, lo, hi, dtype=jnp.int32)
    def uniform(self, shape, lo=0.0, hi=1.0):
        return jax.random.uniform(self._next(), shape, jnp.bfloat16, lo, hi)
    def permutation(self, n):
        return jax.random.permutation(self._next(), n)


kernel_name = 'standalone__linear_kernel_rfa__decode'

def setup_inputs():
    _rng = _Rng(jax.random.key(int.from_bytes(__import__("os").urandom(4), "little")))
    _w = (lambda a: (lambda t: t.astype(jnp.bfloat16) if jnp.issubdtype(t.dtype, jnp.floating) else t)(jnp.asarray(a)))
    B, H, Sq, Sk, D, M = 2, 16, 1, 16384, 256, 16
    return {
        "q": _w((lambda *s: _rng.normal(s) * 0.4)(B, H, Sq, D)),
        "k": _w((lambda *s: _rng.normal(s) * 1.6)(B, H, Sk, D)),
        "v": _w((lambda *s: _rng.normal(s) * 1.6)(B, H, Sk, D)),
        "omega": _w((lambda *s: _rng.normal(s) * 1.6)(M, D)),
    }

def reference(q, k, v, omega):
    d = q.shape[-1]
    m = omega.shape[0]
    scale = float(d) ** -0.25
    qs = q * scale
    ks = k * scale
    q_proj = jnp.einsum("bhsd,md->bhsm", qs, omega)
    k_proj = jnp.einsum("bhsd,md->bhsm", ks, omega)
    q_sq = 0.5 * jnp.einsum("bhsd,bhsd->bhs", qs, qs)[..., None]
    k_sq = 0.5 * jnp.einsum("bhsd,bhsd->bhs", ks, ks)[..., None]
    inv_sqrt_m = float(m) ** -0.5
    phi_q = jnp.exp(q_proj - q_sq) * inv_sqrt_m + 1e-6
    phi_k = jnp.exp(k_proj - k_sq) * inv_sqrt_m + 1e-6
    kv = jnp.einsum("bhsm,bhsd->bhmd", phi_k, v)
    z  = jnp.einsum("bhsm->bhm", phi_k)
    num = jnp.einsum("bhqm,bhmd->bhqd", phi_q, kv)
    den = jnp.einsum("bhqm,bhm->bhq", phi_q, z)[..., None] + 1e-6
    return num / den
```

```python
import functools

import jax
import jax.numpy as jnp
import jax.experimental.pallas as pl
import jax.experimental.pallas.tpu as pltpu

NT = (((1,), (1,)), ((), ()))
sizes = (96, 96, 96, 96, 128)
bk, nbuf, sub = sum(sizes), 8, 512


@jax.jit
def pallas_standalone__linear_kernel_rfa__decode_kernel(
    q: jax.Array, k: jax.Array, v: jax.Array, omega: jax.Array
):
    B, H, Sq, D = q.shape
    Sk = k.shape[2]
    M = omega.shape[0]
    BH = B * H
    scale = float(D) ** -0.25
    inv_sqrt_m = float(M) ** -0.5
    nk = Sk // bk
    total = BH * nk
    csub = min(sub, bk)
    def kern(q_hbm, om_hbm, k_hbm, v_hbm, o_ref, kbuf, vbuf, ksem, vsem, of_ref, q_ref, om_ref, ssem):
        def start(i, slot):
            r = 0
            for p, n in enumerate(sizes):
                off = pl.multiple_of(i * bk + r, 8)
                ck = pltpu.make_async_copy(k_hbm.at[pl.ds(off, n), :], kbuf.at[slot, pl.ds(r, n)], ksem.at[slot])
                cv = pltpu.make_async_copy(v_hbm.at[pl.ds(off, n), :], vbuf.at[slot, pl.ds(r, n)], vsem.at[slot])
                ck.start(priority=p % 2)
                cv.start(priority=(p + 1) % 2)
                r += n

        for s in range(nbuf - 1):
            start(s, s)
        cq = pltpu.make_async_copy(q_hbm, q_ref, ssem.at[0])
        co = pltpu.make_async_copy(om_hbm, om_ref, ssem.at[1])
        cq.start(); co.start(); cq.wait(); co.wait()
        om = (om_ref[...].astype(jnp.float32) * scale).astype(jnp.bfloat16)
        msq = jnp.full((M, 128), -0.5 * scale * scale, jnp.bfloat16)

        def body(i, carry, do_start):
            acc, z = carry
            slot = i % nbuf
            h = i // nk; j = i % nk
            if do_start:
                start(i + nbuf - 1, (i + nbuf - 1) % nbuf)
            pltpu.make_async_copy(kbuf.at[slot], kbuf.at[slot], ksem.at[slot]).wait()
            pltpu.make_async_copy(vbuf.at[slot], vbuf.at[slot], vsem.at[slot]).wait()
            acc = jnp.where(j == 0, 0.0, acc)
            z = jnp.where(j == 0, 0.0, z)
            for c in range(bk // csub):
                kk = kbuf[slot, c*csub:(c+1)*csub, :]
                kf = kk.astype(jnp.float32)
                k2 = kf * kf
                s = (k2[:, :128] + k2[:, 128:]).astype(jnp.bfloat16)
                lg = jax.lax.dot_general(om, kk, NT, preferred_element_type=jnp.float32)
                lg = lg + jax.lax.dot_general(msq, s, NT, preferred_element_type=jnp.float32)
                phi = jnp.exp(lg) * inv_sqrt_m + 1e-6
                for t in range(csub // 128):
                    z = z + phi[:, t*128:(t+1)*128]
                acc = acc + jnp.dot(phi.astype(jnp.bfloat16), vbuf[slot, c*csub:(c+1)*csub, :], preferred_element_type=jnp.float32)

            @pl.when(j == nk - 1)
            def _():
                qa = q_ref[...].astype(jnp.float32) * scale
                rows = jax.lax.broadcasted_iota(jnp.int32, (BH, D), 0)
                qf = jnp.sum(jnp.where(rows == h, qa, 0.0), axis=0, keepdims=True)
                omf = om_ref[...].astype(jnp.float32)
                qp = jnp.sum(omf * qf, axis=1, keepdims=True)
                qsq = 0.5 * jnp.sum(qf * qf, axis=1, keepdims=True)
                phq = jnp.exp(qp - qsq) * inv_sqrt_m + 1e-6
                num = jnp.sum(phq * acc, axis=0, keepdims=True)
                zz = jnp.sum(z, axis=1, keepdims=True)
                den = jnp.sum(phq * zz, axis=0, keepdims=True) + 1e-6
                of_ref[pl.ds(h, 1), :] = num / den
            return acc, z
        carry = (jnp.zeros((M, D), jnp.float32), jnp.zeros((M, 128), jnp.float32))
        nmain = total - (nbuf - 1)
        carry = jax.lax.fori_loop(0, nmain, functools.partial(body, do_start=True), carry)
        carry = jax.lax.fori_loop(nmain, total, functools.partial(body, do_start=False), carry)
        o_ref[...] = of_ref[...].astype(o_ref.dtype)
    out = pl.pallas_call(
        kern,
        in_specs=[pl.BlockSpec(memory_space=pl.ANY), pl.BlockSpec(memory_space=pl.ANY),
                  pl.BlockSpec(memory_space=pl.ANY), pl.BlockSpec(memory_space=pl.ANY)],
        out_specs=pl.BlockSpec(memory_space=pltpu.VMEM),
        out_shape=jax.ShapeDtypeStruct((BH, D), q.dtype),
        scratch_shapes=[pltpu.VMEM((nbuf, bk, D), jnp.bfloat16), pltpu.VMEM((nbuf, bk, D), jnp.bfloat16),
                        pltpu.SemaphoreType.DMA((nbuf,)), pltpu.SemaphoreType.DMA((nbuf,)),
                        pltpu.VMEM((BH, D), jnp.float32), pltpu.VMEM((BH, D), q.dtype), pltpu.VMEM((M, D), omega.dtype), pltpu.SemaphoreType.DMA((2,))],
        compiler_params=pltpu.CompilerParams(vmem_limit_bytes=100 * 1024 * 1024),
    )(q.reshape(BH, D), omega, k.reshape(BH * Sk, D), v.reshape(BH * Sk, D))
    return out.reshape(B, H, Sq, D)
```
